```python
import jax
import jax.numpy as jnp

def _softmax(x, axis=-1):
    return jax.nn.softmax(x, axis=axis)
def _gelu(x):
    return jax.nn.gelu(x, approximate=True)
def _silu(x):
    return jax.nn.silu(x)
def _sigmoid(x):
    return jax.nn.sigmoid(x)
def _layernorm(x, axis=-1, eps=1e-5):
    m = jnp.mean(x, axis=axis, keepdims=True)
    v = jnp.var(x, axis=axis, keepdims=True)
    return (x - m) / jnp.sqrt(v + eps)
def _scatter_add(tgt, idx, src, axis=0):
    return tgt.at[idx].add(src)
def _segment_sum(src, seg, n):
    return jax.ops.segment_sum(src, seg, n)
class _Rng:
    def __init__(self, key):
        self._k = key
    def _next(self):
        self._k, sub = jax.random.split(self._k)
        return sub
    def normal(self, shape):
        return jax.random.normal(self._next(), shape, dtype=jnp.bfloat16)
    def randint(self, lo, hi, shape):
        return jax.random.randint(self._next(), shape, lo, hi, dtype=jnp.int32)
    def uniform(self, shape, lo=0.0, hi=1.0):
        return jax.random.uniform(self._next(), shape, jnp.bfloat16, lo, hi)
    def permutation(self, n):
        return jax.random.permutation(self._next(), n)


kernel_name = 'recurrent_scan__sliding_block_cached__moe_arch_mod__prompt'

def setup_inputs():
    _rng = _Rng(jax.random.key(int.from_bytes(__import__("os").urandom(4), "little")))
    _w = (lambda a: (lambda t: t.astype(jnp.bfloat16) if jnp.issubdtype(t.dtype, jnp.floating) else t)(jnp.asarray(a)))
    def _A_setup():
        B, Sq, D = 1, 2048, 640
        Hq, Hkv, Sk, Dh = 32, 32, 2048, 192
        assert Hq % Hkv == 0, (Hq, Hkv)
        return {
            "x": _w((lambda *s: _rng.normal(s) * 0.05)(B, Sq, D)),
            "k_cache": _w((lambda *s: _rng.normal(s) * 0.05)(B, Hkv, Sk, Dh)),
            "v_cache": _w((lambda *s: _rng.normal(s) * 0.05)(B, Hkv, Sk, Dh)),
            "wq": _w((lambda *s: _rng.normal(s) * 0.05)(D, Hq * Dh) * (D ** -0.5)),
            "wo": _w((lambda *s: _rng.normal(s) * 0.05)(Hq * Dh, D) * ((Hq * Dh) ** -0.5)),
        }
    _A_in = _A_setup()

    def _B_setup():
        B, S, D, F, C = 1, 2048, 640, 1536, 2
        return {
            "x": _w((lambda *s: _rng.normal(s) * 0.05)(B, S, D)),
            "w_r": _w((lambda *s: _rng.normal(s) * 0.05)(D)),
            "w_gate": _w((lambda *s: _rng.normal(s) * 0.05)(D, F)),
            "w_up": _w((lambda *s: _rng.normal(s) * 0.05)(D, F)),
            "w_down": _w((lambda *s: _rng.normal(s) * 0.05)(F, D)),
        }
    _B_in = _B_setup()

    return {
        "A_x": _A_in["x"],
        "A_k_cache": _A_in["k_cache"],
        "A_v_cache": _A_in["v_cache"],
        "A_wq": _A_in["wq"],
        "A_wo": _A_in["wo"],
        "B_x": _B_in["x"],
        "B_w_r": _B_in["w_r"],
        "B_w_gate": _B_in["w_gate"],
        "B_w_up": _B_in["w_up"],
        "B_w_down": _B_in["w_down"],
    }

def reference(A_x, A_k_cache, A_v_cache, A_wq, A_wo, B_x, B_w_r, B_w_gate, B_w_up, B_w_down):
    def _A_ref(x, k_cache, v_cache, wq, wo):
        B, Sq, D = x.shape
        Hq, Dh = 32, 192
        Hkv, Sk = k_cache.shape[1], k_cache.shape[2]
        W = min(4096, max(256, Sk // 4))
        rep = Hq // Hkv
        q = (lambda x, *d: x.transpose(*d))((x @ wq).reshape(B, Sq, Hq, Dh), 0, 2, 1, 3)
        k = jnp.repeat(k_cache[:, :, Sk - W:, :], rep, axis=1)
        v = jnp.repeat(v_cache[:, :, Sk - W:, :], rep, axis=1)
        scores = jnp.einsum("bhqd,bhkd->bhqk", q, k) * (Dh ** -0.5)
        p = _softmax(scores, axis=-1)
        o = jnp.einsum("bhqk,bhkd->bhqd", p, v)
        return (lambda x, *d: x.transpose(*d))(o, 0, 2, 1, 3).reshape(B, Sq, Hq * Dh) @ wo

    def _B_ref(x, w_r, w_gate, w_up, w_down):
        B, S, D = x.shape
        C = 2
        r = x @ w_r
        idx = jnp.argsort(-r, axis=-1)[:, :C]
        idx_e = jnp.repeat(idx.reshape(B, C, 1), D, axis=2)
        x_sel = jnp.take_along_axis(x, idx_e, axis=1)
        g = _silu(x_sel @ w_gate)
        u = x_sel @ w_up
        y = (g * u) @ w_down
        r_sel = _sigmoid(jnp.take_along_axis(r, idx, axis=1))
        y = y * r_sel.reshape(B, C, 1)
        b_off = (jnp.arange(B) * S).reshape(B, 1)
        flat_idx = (idx + b_off).reshape(B * C)
        zero = (x * 0.0).reshape(B * S, D)
        upd = _scatter_add(zero, flat_idx, y.reshape(B * C, D), axis=0)
        return x + upd.reshape(B, S, D)

    x = A_x
    xn = _layernorm(x, axis=-1)
    s = _A_ref(xn, A_k_cache, A_v_cache, A_wq, A_wo)
    g = _silu(_B_ref(xn, B_w_r, B_w_gate, B_w_up, B_w_down))
    return x + s * g
```

```python
import jax
import jax.numpy as jnp
from jax import lax
from jax.experimental import pallas as pl
from jax.experimental.pallas import tpu as pltpu

F32 = jnp.float32
BF16 = jnp.bfloat16
U32 = jnp.uint32
I32 = jnp.int32
LOG2E = 1.4426950408889634

S, D = 2048, 640
H, DH, W = 32, 192, 512
FF = 1536
EPS = 1e-5
HB = 64
KH = W // 2
PW = 2 * DH
NPAIR = H // 2
M = 256
NQ = S // M
NN = M // 128
DL = D // 2


def _pack(x):
    return pltpu.bitcast(x, U32)


def _unpack(x):
    return pltpu.bitcast(x, BF16)


def _bf(x):
    n = x.shape[1] // 128
    if n <= 1:
        return x.astype(BF16)
    parts = [pltpu.bitcast(x[:, i * 128:(i + 1) * 128].astype(BF16), U32) for i in range(n)]
    return pltpu.bitcast(jnp.concatenate(parts, axis=1), BF16)


def _ipack(a, b):
    return pltpu.pack_elementwise([a, b], packed_dtype=BF16)


def _iunpack(u):
    return (pltpu.unpack_elementwise(u, index=0, packed_dtype=BF16, unpacked_dtype=F32),
            pltpu.unpack_elementwise(u, index=1, packed_dtype=BF16, unpacked_dtype=F32))


def _interleave(a, b):
    return _unpack(_ipack(a, b)).astype(F32)


def _par(p):
    return p & 1


def _sigmoid(x):
    return 0.5 * jnp.tanh(0.5 * x) + 0.5


def _rb(x):
    return x.astype(BF16).astype(F32)


def _recip(l):
    r = pl.reciprocal(l, approx=True)
    return r * (2.0 - l * r)


def _dot(a, b):
    return jnp.dot(a, b, preferred_element_type=F32)


def _fold(x, op):
    parts = [x[i:i + 8] for i in range(0, x.shape[0], 8)]
    while len(parts) > 1:
        nxt = [op(parts[i], parts[i + 1]) for i in range(0, len(parts) - 1, 2)]
        if len(parts) % 2:
            nxt.append(parts[-1])
        parts = nxt
    return parts[0]


def _strassen_a(a11, a12, a21, a22):
    return [a11 + a22, a21 + a22, a11, a22, a11 + a12, a21 - a11, a12 - a22]


def _strassen_b(b11, b12, b21, b22):
    return [b11 + b22, b11, b12 - b22, b21 - b11, b22, b11 + b12, b21 + b22]


def _strassen_c(m):
    m1, m2, m3, m4, m5, m6, m7 = m
    return m1 + m4 - m5 + m7, m3 + m5, m2 + m4, m1 - m2 + m3 + m6


def make_kernel(cfg):
    cfg = cfg or {}
    npair = cfg.get("npair", NPAIR)
    G = cfg.get("ng", 4)
    S1, S2 = cfg.get("s1", True), cfg.get("s2", True)
    sched = cfg.get("sched", "end")
    gr = KH // G
    PINS = cfg.get("pins", {7: [0]})
    qscale = (DH ** -0.5) * LOG2E

    def kernel(x_hbm, kt_hbm, vt_hbm, wq_hbm, wo_hbm, wr_ref, wg_hbm, wu_hbm, wd_hbm,
               out_hbm,
               x_buf, xt_ref, xn_ref, sx_ref, acc_ref, wq_buf, wo_buf, kt_buf, vt_buf,
               wqs_ref, wq4_ref, ks_ref, vs_ref, wos_ref, wo1_ref, qc_ref, oc_ref, r_ref, upd_ref, idx_ref,
               wg_buf, wu_buf, wd_buf, out_buf, tmp_ref, pe_ref,
               sem_x, sem_w, sem_f, sem_o):
        j = pl.program_id(0)
        sk = kt_hbm.shape[3]

        def cp_x(i):
            return pltpu.make_async_copy(x_hbm.at[pl.ds(i * M, M), :], x_buf.at[pl.ds(i * M, M), :], sem_x.at[i])

        def _off(p, n):
            return p * n if isinstance(p, int) else pl.multiple_of(p * n, 128)

        def cp_w(p):
            sl = _par(p)
            return [
                pltpu.make_async_copy(wq_hbm.at[:, pl.ds(_off(p, PW), PW)], wq_buf.at[sl], sem_w.at[sl]),
                pltpu.make_async_copy(kt_hbm.at[0, pl.ds(2 * p, 2), :, pl.ds(sk - W, W)], kt_buf.at[sl], sem_w.at[2 + sl]),
                pltpu.make_async_copy(vt_hbm.at[0, pl.ds(2 * p, 2), :, pl.ds(sk - W, W)], vt_buf.at[sl], sem_w.at[4 + sl]),
                pltpu.make_async_copy(wo_hbm.at[pl.ds(_off(p, PW), PW), :], wo_buf.at[sl], sem_w.at[6 + sl]),
            ]

        def cp_f(k):
            src, dst = [(wg_hbm, wg_buf), (wu_hbm, wu_buf), (wd_hbm, wd_buf)][k]
            return pltpu.make_async_copy(src, dst, sem_f.at[k])

        def cp_out(i):
            return pltpu.make_async_copy(out_buf.at[pl.ds(i * M, M), :], out_hbm.at[pl.ds(i * M, M), :], sem_o.at[i])

        def cols(b, n=None):
            off, sz = (b * M, M) if n is None else (b * M + n * 128, 128)
            return pl.ds(off if isinstance(b, int) else pl.multiple_of(off, 128), sz)

        def layernorm(b):
            xt = _pack(x_buf[cols(b), :]).T
            xt_ref[b] = xt
            wr = wr_ref[...].astype(F32)
            halves = []
            stats = []
            for x in _iunpack(xt):
                piv = x[0:1]
                xs = x - piv
                m1 = jnp.sum(_fold(xs, jnp.add), axis=0, keepdims=True) * (1.0 / D)
                m2 = jnp.sum(_fold(xs * xs, jnp.add), axis=0, keepdims=True) * (1.0 / D)
                var = jnp.maximum(m2 - m1 * m1, 0.0)
                stats.append((piv + m1, lax.rsqrt(var + EPS)))
            b2 = b if isinstance(b, int) else (b + NQ) % NQ
            for n, x in enumerate(_iunpack(xt_ref[b2])):
                xn = (x - stats[n][0]) * stats[n][1]
                u = _ipack(xn[:DL], xn[DL:])
                xn_ref[:, cols(b, n)] = u
                lo, hi = _iunpack(u)
                r = jnp.sum(_fold(lo * wr[:DL] + hi * wr[DL:], jnp.add), axis=0, keepdims=True)
                r_ref[:, cols(b, n)] = _rb(r)
                halves.append((lo, hi))
            if S1:
                cs = [_strassen_b(halves[0][i][:128], halves[1][i][:128], halves[0][i][128:256], halves[1][i][128:256])
                      for i in range(2)]
                for t, i in enumerate((0, 2, 3, 5, 6)):
                    sx_ref[b, t] = _ipack(cs[0][i], cs[1][i])

        def stage_wq(p):
            sl = _par(p)
            w = wq_buf[sl].astype(F32)
            wt = _interleave(w[:DL], w[DL:]).T
            if S1:
                a = _strassen_a(wt[:DH, :256], wt[:DH, 256:512], wt[DH:, :256], wt[DH:, 256:512])
                for i in range(7):
                    wqs_ref[sl, i] = _pack(_bf(a[i]))
                wq4_ref[sl] = _pack(_bf(wt[:, 512:]))
            else:
                wq4_ref[sl] = _pack(_bf(wt[:, 512:]))
                for i, (r0, c0) in enumerate([(0, 0), (0, 256), (DH, 0), (DH, 256)]):
                    wqs_ref[sl, i] = _pack(_bf(wt[r0:r0 + DH, c0:c0 + 256]))

        def stage_k(p, h, t):
            sl = _par(p)

            def blk(b, half):
                return kt_buf[sl, h, b * HB:(b + 1) * HB, half * KH:(half + 1) * KH].astype(F32)
            top, bot = [lambda: (blk(0, 1), blk(1, 0) + blk(1, 1)),
                        lambda: (blk(0, 0), blk(2, 0) + blk(2, 1)),
                        lambda: (blk(1, 0), -blk(2, 1))][t]()
            tmp_ref[...] = _interleave(top, bot).T
            for c in range(KH // 32):
                ld = [tmp_ref[pl.ds(c * 32 + o, 8, stride=4), :] for o in range(4)]
                ks_ref[sl, h, t, c * 16:(c + 1) * 16, :] = _ipack(
                    jnp.concatenate(ld[:2], axis=0), jnp.concatenate(ld[2:], axis=0))

        def stage_v(p, h):
            vs_ref[_par(p), h] = _pack(vt_buf[_par(p), h])

        def stage_wo(p):
            sl = _par(p)
            w = wo_buf[sl].astype(F32)
            wt = _interleave(w[:DH], w[DH:]).T
            wo1_ref[sl] = _pack(wt[:, 128:256].astype(BF16))
            if S2:
                a = _strassen_a(wt[:DL, :128], wt[:DL, 256:], wt[DL:, :128], wt[DL:, 256:])
                for i in range(7):
                    wos_ref[sl, i] = _pack(a[i].astype(BF16))
            else:
                for i, (r0, c0) in enumerate([(0, 0), (0, 256), (DL, 0), (DL, 256)]):
                    wos_ref[sl, i] = _pack(wt[r0:r0 + DL, c0:c0 + 128].astype(BF16))

        def stage_all(p):
            stage_wq(p)
            for h in range(2):
                for t in range(3):
                    stage_k(p, h, t)
                stage_v(p, h)
            stage_wo(p)

        def qproj(b, p):
            sl = _par(p)
            xn = xn_ref[:, cols(b)]
            k4 = _dot(_unpack(wq4_ref[sl]), _unpack(xn[256:]))
            if S1:
                def xb(kh, n):
                    return xn[kh * 128:(kh + 1) * 128, n * 128:(n + 1) * 128]
                bs = [sx_ref[b, 0], xb(0, 0), sx_ref[b, 1], sx_ref[b, 2], xb(1, 1), sx_ref[b, 3], sx_ref[b, 4]]
                mm = [_dot(_unpack(wqs_ref[sl, i]), _unpack(bs[i])) for i in range(7)]
                c11, c12, c21, c22 = _strassen_c(mm)
                qa = jnp.concatenate([c11, c12], axis=1)
                qb = jnp.concatenate([c21, c22], axis=1)
            else:
                x1, x2 = _unpack(xn[:128]), _unpack(xn[128:256])
                qa = _dot(_unpack(wqs_ref[sl, 0]), x1) + _dot(_unpack(wqs_ref[sl, 1]), x2)
                qb = _dot(_unpack(wqs_ref[sl, 2]), x1) + _dot(_unpack(wqs_ref[sl, 3]), x2)
            ops = []
            for h, qh in enumerate((qa, qb)):
                qh = (qh + k4[h * DH:(h + 1) * DH]) * qscale
                u, v, w = (qh[t * HB:(t + 1) * HB] for t in range(3))
                ops += [_ipack(u, v), _ipack(u, w), _ipack(v, w)]
            return ops

        def qk_softmax(X, h, p):
            sl = _par(p)
            xuv, xuw, xvw = X[3 * h:3 * h + 3]
            res = []
            for n in range(NN):
                c = slice(n * 128, (n + 1) * 128)
                wuw, wvw, wuv = _unpack(xuw[:, c]), _unpack(xvw[:, c]), _unpack(xuv[:, c])
                m = None
                es, ms, ls = [], [], []
                for g in range(G):
                    rr = slice(g * gr // 2, (g + 1) * gr // 2)
                    a = _dot(_unpack(ks_ref[sl, h, 1, rr, :]), wuw)
                    bb = _dot(_unpack(ks_ref[sl, h, 2, rr, :]), wvw)
                    cc = _dot(_unpack(ks_ref[sl, h, 0, rr, :]), wuv)
                    sL = a + bb
                    sR = cc - bb
                    mg = jnp.max(_fold(jnp.maximum(sL, sR), jnp.maximum), axis=0, keepdims=True)
                    m = mg if m is None else jnp.maximum(m, mg)
                    parts, acc = [], None
                    for sc in (sL, sR):
                        for r in range(0, gr, 32):
                            e = jnp.exp2(sc[r:r + 32] - m)
                            parts.append(_ipack(e[:16], e[16:]))
                            e8 = _fold(e, jnp.add)
                            acc = e8 if acc is None else acc + e8
                    if cfg.get("p_ref"):
                        pe_ref[j % 2, h, n, g * gr:(g + 1) * gr, :] = jnp.concatenate(parts, axis=0)
                        es.append(None)
                    else:
                        es.append(jnp.concatenate(parts, axis=0))
                    ms.append(m)
                    ls.append(acc)
                res.append((es, ms, ls))
            return res

        def pv(res, h, p):
            v = _unpack(vs_ref[_par(p), h])
            outs = []
            for n in range(NN):
                es, ms, ls = res[n]
                o, l = None, None
                for g in range(G):
                    vg = jnp.concatenate([v[:, g * gr:(g + 1) * gr], v[:, KH + g * gr:KH + (g + 1) * gr]], axis=1)
                    eg = pe_ref[1 - (j + 1) % 2, h, n, g * gr:(g + 1) * gr, :] if cfg.get("p_ref") else es[g]
                    d = _dot(vg, _unpack(eg))
                    if o is None:
                        o, l = d, ls[g]
                    else:
                        al = jnp.exp2(ms[g - 1] - ms[g])
                        o = o * al + d
                        l = l * al + ls[g]
                outs.append(o * _recip(jnp.sum(l, axis=0, keepdims=True)))
            return outs

        NO = 9 if S2 else 6

        def fin(oa, ob):
            def blk(x, t, n):
                return x[n][t * HB:(t + 1) * HB]
            mid = [_ipack(blk(oa, 1, n), blk(ob, 1, n)) for n in range(NN)]
            if S2:
                ca = _strassen_b(blk(oa, 0, 0), blk(oa, 0, 1), blk(oa, 2, 0), blk(oa, 2, 1))
                cb = _strassen_b(blk(ob, 0, 0), blk(ob, 0, 1), blk(ob, 2, 0), blk(ob, 2, 1))
                return [_ipack(ca[i], cb[i]) for i in range(7)] + mid
            return [_ipack(blk(oa, t, n), blk(ob, t, n)) for t in (0, 2) for n in range(NN)] + mid

        def wo_y(os, p):
            sl = _par(p)
            w1 = _unpack(wo1_ref[sl])
            mid = [_dot(w1, _unpack(os[-NN + n])) for n in range(NN)]
            if S2:
                mm = [_dot(_unpack(wos_ref[sl, i]), _unpack(os[i])) for i in range(7)]
                c11, c12, c21, c22 = _strassen_c(mm)
            else:
                w = [_unpack(wos_ref[sl, i]) for i in range(4)]
                b11, b12, b21, b22 = (_unpack(o) for o in os[:4])
                c11 = _dot(w[0], b11) + _dot(w[1], b21)
                c12 = _dot(w[0], b12) + _dot(w[1], b22)
                c21 = _dot(w[2], b11) + _dot(w[3], b21)
                c22 = _dot(w[2], b12) + _dot(w[3], b22)
            return [jnp.concatenate([c11, c21], axis=0) + mid[0], jnp.concatenate([c12, c22], axis=0) + mid[1]]

        def wo(b, os, p):
            y = wo_y(os, p)
            for n in range(NN):
                acc_ref[:, cols(b, n)] += y[n]

        def epilogue(b, y):
            xs = _iunpack(xt_ref[b])
            outs = []
            for n in range(NN):
                xn = jnp.concatenate(_iunpack(xn_ref[:, cols(b, n)]), axis=0)
                qid = b * M + 2 * lax.broadcasted_iota(I32, (1, 128), 1) + n
                hh = xn + jnp.where(qid == idx_ref[0:1, 0:1], upd_ref[0], jnp.where(qid == idx_ref[1:2, 0:1], upd_ref[1], 0.0))
                h2 = 0.5 * hh
                g = h2 * jnp.tanh(h2) + h2
                outs.append(xs[n] + (acc_ref[:, cols(b, n)] + y[n]) * g)
            out_buf[cols(b), :] = _unpack(_ipack(outs[0], outs[1]).T)
            cp_out(b).start()

        def router_ffn():
            r = r_ref[...]
            col = lax.broadcasted_iota(I32, (1, S), 1)
            cid = (col // M) * M + 2 * (col % 128) + (col // 128) % 2
            m1 = jnp.max(r, axis=1, keepdims=True)
            i1 = jnp.min(jnp.where(r == m1, cid, S), axis=1, keepdims=True)
            r2 = jnp.where(cid == i1, -jnp.inf, r)
            m2 = jnp.max(r2, axis=1, keepdims=True)
            i2 = jnp.min(jnp.where(jnp.logical_and(r2 == m2, cid != i1), cid, S), axis=1, keepdims=True)
            i1 = jnp.minimum(i1, S - 1)
            i2 = jnp.minimum(i2, S - 1)

            def gather(iv):
                sc = jnp.min(iv)
                base = pl.multiple_of((sc // 16) * 16, 16)
                blk = x_buf[pl.ds(base, 16), :].astype(F32)
                sub = lax.broadcasted_iota(I32, (16, 1), 0)
                xr = jnp.sum(jnp.where(sub == sc % 16, blk, 0.0), axis=0, keepdims=True)
                mu = jnp.sum(xr, axis=1, keepdims=True) * (1.0 / D)
                xc = xr - mu
                var = jnp.sum(xc * xc, axis=1, keepdims=True) * (1.0 / D)
                return xc * lax.rsqrt(var + EPS)
            row = lax.broadcasted_iota(I32, (16, 1), 0)
            xs = jnp.where(row == 0, gather(i1), jnp.where(row == 1, gather(i2), 0.0)).astype(BF16)
            g = _rb(_dot(xs, wg_buf[...]))
            g = _rb(g * _sigmoid(g))
            u = _rb(_dot(xs, wu_buf[...]))
            gu = (g * u).astype(BF16)
            y = _rb(_dot(gu, wd_buf[...]))
            rs = _rb(_sigmoid(jnp.where(row == 0, m1, m2)))
            upd = _rb(y * rs)
            updt = jnp.concatenate([upd, jnp.zeros((112, D), F32)], axis=0).T
            for t in range(2):
                upd_ref[t] = jnp.broadcast_to(updt[:, t:t + 1], (D, 128))
            idx_ref[...] = jnp.broadcast_to(jnp.where(row == 0, i1, i2), (16, 128))

        @pl.when(j == 0)
        def _():
            w0, w1 = cp_w(0), cp_w(1)
            cp_x(0).start(); w0[0].start()
            for i in range(1, NQ): cp_x(i).start()
            w0[1].start()
            acc_ref[...] = jnp.zeros(acc_ref.shape, F32)
            oc_ref[...] = jnp.zeros(oc_ref.shape, U32)
            wos_ref[1] = jnp.zeros(wos_ref.shape[1:], U32)
            wo1_ref[1] = jnp.zeros(wo1_ref.shape[1:], U32)
            cp_x(0).wait()
            w0[2].start(); w0[3].start()
            for c in w1: c.start()
            layernorm(0)
            w0[0].wait(); stage_wq(0)
            X0 = qproj(0, 0)
            for t in range(6): qc_ref[t] = X0[t]
            cp_x(1).wait(); layernorm(1)

            def ln(i, c):
                cp_x(i).wait(); layernorm(i)
                return c
            lax.fori_loop(2, NQ, ln, 0)
            for k in range(3): cp_f(k).start()
            w0[1].wait()
            for h in range(2):
                for t in range(3): stage_k(0, h, t)
            w0[2].wait(); stage_v(0, 0); stage_v(0, 1)
            w0[3].wait(); stage_wo(0)

        @pl.when(j + 1 < npair)
        def _():
            for c in cp_w(j + 1): c.wait()

        @pl.when(j + 2 < npair)
        def _():
            for c in cp_w(j + 2): c.start()

        @pl.when(j == 1)
        def _():
            for k in range(3): cp_f(k).wait()
            router_ffn()

        def body(last_step):
            X = [qc_ref[t] for t in range(6)]
            o_prev = [oc_ref[t] for t in range(NO)]
            for i in range(NQ):
                last = i == NQ - 1
                ra = qk_softmax(X, 0, j)
                if i == 0:
                    wo(NQ - 1, o_prev, j + 1)
                elif last_step:
                    epilogue(i - 1, wo_y(o_prev, j))
                    if i in PINS:
                        for bb in PINS[i]:
                            cp_out(bb).wait()
                else:
                    wo(i - 1, o_prev, j)
                rb = qk_softmax(X, 1, j)
                if last and not last_step:
                    stage_wq(j + 1); stage_wo(j + 1)
                    for h in range(2):
                        for t in range(3): stage_k(j + 1, h, t)
                oa = pv(ra, 0, j)
                if not last:
                    X = qproj(i + 1, j)
                elif not last_step:
                    Xn = qproj(0, j + 1)
                    for t in range(6): qc_ref[t] = Xn[t]
                ob = pv(rb, 1, j)
                o_prev = fin(oa, ob)
            if last_step:
                epilogue(NQ - 1, wo_y(o_prev, j))
                waited = [bb for v in PINS.values() for bb in v]
                for i in range(NQ):
                    if i not in waited:
                        cp_out(i).wait()
            else:
                stage_v(j + 1, 0); stage_v(j + 1, 1)
                for t in range(NO): oc_ref[t] = o_prev[t]

        @pl.when(j < npair - 1)
        def _():
            body(False)

        @pl.when(j == npair - 1)
        def _():
            body(True)

    return kernel, npair, NO_of(S2)


def NO_of(s2):
    return 9 if s2 else 6


def _impl(cfg, A_x, A_k_cache, A_v_cache, A_wq, A_wo, B_x, B_w_r, B_w_gate, B_w_up, B_w_down):
    cfg = cfg or {}
    S1, S2 = cfg.get("s1", True), cfg.get("s2", True)
    if True:
        x = A_x.reshape(S, D)
        kt = jnp.swapaxes(A_k_cache, 2, 3)
        vt = jnp.swapaxes(A_v_cache, 2, 3)
        wr = B_w_r.reshape(D, 1)
        anyspec = pl.BlockSpec(memory_space=pl.ANY)
        kernel, ns, no = make_kernel(cfg)
        out = pl.pallas_call(
            kernel,
            grid=(ns,),
            in_specs=[anyspec, anyspec, anyspec, anyspec, anyspec,
                      pl.BlockSpec((D, 1), lambda j: (0, 0)),
                      anyspec, anyspec, anyspec],
            out_specs=anyspec,
            out_shape=jax.ShapeDtypeStruct((S, D), BF16),
            scratch_shapes=[
                pltpu.VMEM((S, D), BF16),
                pltpu.VMEM((NQ, D, 128), U32),
                pltpu.VMEM((DL, S), U32),
                pltpu.VMEM((NQ, 5, 128, 128), U32),
                pltpu.VMEM((D, S), F32),
                pltpu.VMEM((2, D, PW), BF16),
                pltpu.VMEM((2, PW, D), BF16),
                pltpu.VMEM((2, 2, DH, W), BF16),
                pltpu.VMEM((2, 2, DH, W), BF16),
                pltpu.VMEM((2, 7 if S1 else 4, DH // 2, 256), U32),
                pltpu.VMEM((2, PW // 2, 128), U32),
                pltpu.VMEM((2, 2, 3, KH // 2, 128), U32),
                pltpu.VMEM((2, 2, DH // 2, W), U32),
                pltpu.VMEM((2, 7 if S2 else 4, DL // 2, 128), U32),
                pltpu.VMEM((2, DL, 128), U32),
                pltpu.VMEM((6, HB, M), U32),
                pltpu.VMEM((no, HB, 128), U32),
                pltpu.VMEM((1, S), F32),
                pltpu.VMEM((2, D, 128), F32),
                pltpu.VMEM((16, 128), I32),
                pltpu.VMEM((D, FF), BF16),
                pltpu.VMEM((D, FF), BF16),
                pltpu.VMEM((FF, D), BF16),
                pltpu.VMEM((S, D), BF16),
                pltpu.VMEM((KH, 128), F32),
                pltpu.VMEM((2, 2, 2, KH, 128), U32),
                pltpu.SemaphoreType.DMA((NQ,)),
                pltpu.SemaphoreType.DMA((8,)),
                pltpu.SemaphoreType.DMA((3,)),
                pltpu.SemaphoreType.DMA((NQ,)),
            ],
            compiler_params=pltpu.CompilerParams(
                dimension_semantics=("arbitrary",),
                vmem_limit_bytes=100 * 1024 * 1024,
                disable_bounds_checks=cfg.get('nobc', True)),
            name="fused_attn_mod",
        )(x, kt, vt, A_wq, A_wo, wr, B_w_gate, B_w_up, B_w_down)
        return out.reshape(1, S, D)


@jax.jit
def pallas_recurrent_scan__sliding_block_cached__moe_arch_mod__prompt_kernel(A_x, A_k_cache, A_v_cache, A_wq, A_wo, B_x, B_w_r, B_w_gate, B_w_up, B_w_down):
    return _impl(None, A_x, A_k_cache, A_v_cache, A_wq, A_wo, B_x, B_w_r, B_w_gate, B_w_up, B_w_down)
```

```python
import jax
import jax.numpy as jnp
from jax import lax
from jax.experimental import pallas as pl
from jax.experimental.pallas import tpu as pltpu

F32 = jnp.float32
BF16 = jnp.bfloat16
U32 = jnp.uint32
I32 = jnp.int32
LOG2E = 1.4426950408889634

S, D = 2048, 640
H, DH, W = 32, 192, 512
FF = 1536
EPS = 1e-5
HB = 64
KH = W // 2
PW = 2 * DH
NPAIR = H // 2
M = 256
NQ = S // M
NN = M // 128
DL = D // 2
G = 4
GR = KH // G
NO = 9


def _pack(x):
    return pltpu.bitcast(x, U32)


def _unpack(x):
    return pltpu.bitcast(x, BF16)


def _bf(x):
    parts = [pltpu.bitcast(x[:, i * 128:(i + 1) * 128].astype(BF16), U32) for i in range(x.shape[1] // 128)]
    return pltpu.bitcast(jnp.concatenate(parts, axis=1), BF16)


def _ipack(a, b):
    return pltpu.pack_elementwise([a, b], packed_dtype=BF16)


def _iunpack(u):
    return (pltpu.unpack_elementwise(u, index=0, packed_dtype=BF16, unpacked_dtype=F32),
            pltpu.unpack_elementwise(u, index=1, packed_dtype=BF16, unpacked_dtype=F32))


def _interleave(a, b):
    return _unpack(_ipack(a, b)).astype(F32)


def _par(p):
    return p & 1


def _sigmoid(x):
    return 0.5 * jnp.tanh(0.5 * x) + 0.5


def _rb(x):
    return x.astype(BF16).astype(F32)


def _recip(l):
    r = pl.reciprocal(l, approx=True)
    return r * (2.0 - l * r)


def _dot(a, b):
    return jnp.dot(a, b, preferred_element_type=F32)


def _fold(x, op):
    parts = [x[i:i + 8] for i in range(0, x.shape[0], 8)]
    while len(parts) > 1:
        nxt = [op(parts[i], parts[i + 1]) for i in range(0, len(parts) - 1, 2)]
        if len(parts) % 2:
            nxt.append(parts[-1])
        parts = nxt
    return parts[0]


def _strassen_a(a11, a12, a21, a22):
    return [a11 + a22, a21 + a22, a11, a22, a11 + a12, a21 - a11, a12 - a22]


def _strassen_b(b11, b12, b21, b22):
    return [b11 + b22, b11, b12 - b22, b21 - b11, b22, b11 + b12, b21 + b22]


def _strassen_c(m):
    m1, m2, m3, m4, m5, m6, m7 = m
    return m1 + m4 - m5 + m7, m3 + m5, m2 + m4, m1 - m2 + m3 + m6


def _kernel(x_hbm, kt_hbm, vt_hbm, wq_hbm, wo_hbm, wr_hbm, wg_hbm, wu_hbm, wd_hbm,
            out_hbm,
            x_buf, xt_ref, xn_ref, sx_ref, acc_ref, wq_buf, wo_buf, kt_buf, vt_buf,
            wqs_ref, wq4_ref, ks_ref, vs_ref, wos_ref, wo1_ref, qc_ref, oc_ref, r_ref, tile_ref,
            wg_buf, wu_buf, wd_buf, out_buf, tmp_ref, wrc_ref, wr_ref,
            sem_x, sem_w, sem_f, sem_o, sem_r):
    j = pl.program_id(0)
    sk = kt_hbm.shape[3]
    qscale = (DH ** -0.5) * LOG2E

    def cp_x(i):
        return pltpu.make_async_copy(x_hbm.at[cols(i), :], x_buf.at[cols(i), :], sem_x.at[i])

    def cp_w(p):
        sl = _par(p)
        off = p * PW if isinstance(p, int) else pl.multiple_of(p * PW, 128)
        return [
            pltpu.make_async_copy(wq_hbm.at[:, pl.ds(off, PW)], wq_buf.at[sl], sem_w.at[sl]),
            pltpu.make_async_copy(kt_hbm.at[0, pl.ds(2 * p, 2), :, pl.ds(sk - W, W)], kt_buf.at[sl], sem_w.at[2 + sl]),
            pltpu.make_async_copy(wo_hbm.at[pl.ds(off, PW), :], wo_buf.at[sl], sem_w.at[6 + sl]),
            pltpu.make_async_copy(vt_hbm.at[0, pl.ds(2 * p, 2), :, pl.ds(sk - W, W)], vt_buf.at[sl], sem_w.at[4 + sl]),
        ]

    def cp_f(k):
        src, dst = [(wg_hbm, wg_buf), (wu_hbm, wu_buf), (wd_hbm, wd_buf)][k]
        return pltpu.make_async_copy(src, dst, sem_f.at[k])

    def cp_out(i):
        return pltpu.make_async_copy(out_buf.at[cols(i), :], out_hbm.at[cols(i), :], sem_o.at[i])

    def cols(b, n=None):
        off, sz = (b * M, M) if n is None else (b * M + n * 128, 128)
        return pl.ds(off if isinstance(b, int) else pl.multiple_of(off, 128), sz)

    def layernorm(b):
        xt = _pack(x_buf[cols(b), :]).T
        xt_ref[b] = xt
        piv = _iunpack(xt[0:1])
        s1, s2 = [[None] * 4, [None] * 4], [[None] * 4, [None] * 4]
        for g in range(D // 8):
            for n, x in enumerate(_iunpack(xt[g * 8:(g + 1) * 8])):
                xs = x - piv[n]
                a = g % 4
                s1[n][a] = xs if s1[n][a] is None else s1[n][a] + xs
                s2[n][a] = xs * xs if s2[n][a] is None else s2[n][a] + xs * xs
        mean, rstd = [], []
        for n in range(2):
            m1 = jnp.sum((s1[n][0] + s1[n][1]) + (s1[n][2] + s1[n][3]), axis=0, keepdims=True) * (1.0 / D)
            m2 = jnp.sum((s2[n][0] + s2[n][1]) + (s2[n][2] + s2[n][3]), axis=0, keepdims=True) * (1.0 / D)
            mean.append(piv[n] + m1)
            rstd.append(lax.rsqrt(jnp.maximum(m2 - m1 * m1, 0.0) + EPS))
        b2 = b if isinstance(b, int) else (b + NQ) % NQ
        racc = [None, None]

        def norm_group(g):
            xl = _iunpack(xt_ref[b2, g * 8:(g + 1) * 8, :])
            xh = _iunpack(xt_ref[b2, DL + g * 8:DL + (g + 1) * 8, :])
            res = []
            for n in range(2):
                u = _ipack((xl[n] - mean[n]) * rstd[n], (xh[n] - mean[n]) * rstd[n])
                xn_ref[g * 8:(g + 1) * 8, cols(b, n)] = u
                lo, hi = _iunpack(u)
                t = lo * wrc_ref[g * 8:(g + 1) * 8, :] + hi * wrc_ref[DL + g * 8:DL + (g + 1) * 8, :]
                racc[n] = t if racc[n] is None else racc[n] + t
                res.append((lo, hi))
            return res
        for g in range(16):
            top, bot = norm_group(g), norm_group(g + 16)
            cs = [_strassen_b(top[0][i], top[1][i], bot[0][i], bot[1][i]) for i in range(2)]
            for t, i in enumerate((0, 2, 3, 5, 6)):
                sx_ref[b, t, g * 8:(g + 1) * 8, :] = _ipack(cs[0][i], cs[1][i])
        for g in range(32, DL // 8):
            norm_group(g)
        for n in range(2):
            r_ref[:, cols(b, n)] = _rb(jnp.sum(racc[n], axis=0, keepdims=True))

    def stage_wq(p):
        sl = _par(p)
        w = wq_buf[sl].astype(F32)
        wt = _interleave(w[:DL], w[DL:]).T
        a = _strassen_a(wt[:DH, :256], wt[:DH, 256:512], wt[DH:, :256], wt[DH:, 256:512])
        for i in range(7):
            wqs_ref[sl, i] = _pack(_bf(a[i]))
        wq4_ref[sl] = _pack(_bf(wt[:, 512:]))

    def stage_k(p, h, t):
        sl = _par(p)

        def blk(b, half):
            return kt_buf[sl, h, b * HB:(b + 1) * HB, half * KH:(half + 1) * KH].astype(F32)
        top, bot = [lambda: (blk(0, 1), blk(1, 0) + blk(1, 1)),
                    lambda: (blk(0, 0), blk(2, 0) + blk(2, 1)),
                    lambda: (blk(1, 0), -blk(2, 1))][t]()
        tmp_ref[...] = _interleave(top, bot).T
        for c in range(KH // 32):
            ld = [tmp_ref[pl.ds(c * 32 + o, 8, stride=4), :] for o in range(4)]
            ks_ref[sl, h, t, c * 16:(c + 1) * 16, :] = _ipack(
                jnp.concatenate(ld[:2], axis=0), jnp.concatenate(ld[2:], axis=0))

    def stage_v(p, h):
        v = _pack(vt_buf[_par(p), h])
        for g in range(G):
            vs_ref[_par(p), h, g] = jnp.concatenate(
                [v[:, g * GR:(g + 1) * GR], v[:, KH + g * GR:KH + (g + 1) * GR]], axis=1)

    def stage_wo(p):
        sl = _par(p)
        w = wo_buf[sl].astype(F32)
        wt = _interleave(w[:DH], w[DH:]).T
        wo1_ref[sl] = _pack(wt[:, 128:256].astype(BF16))
        a = _strassen_a(wt[:DL, :128], wt[:DL, 256:], wt[DL:, :128], wt[DL:, 256:])
        for i in range(7):
            wos_ref[sl, i] = _pack(a[i].astype(BF16))

    def qproj(b, p):
        sl = _par(p)
        xn = xn_ref[:, cols(b)]
        k4 = _dot(_unpack(wq4_ref[sl]), _unpack(xn[256:]))
        bs = [sx_ref[b, 0], xn[:128, :128], sx_ref[b, 1], sx_ref[b, 2], xn[128:256, 128:], sx_ref[b, 3], sx_ref[b, 4]]
        c11, c12, c21, c22 = _strassen_c([_dot(_unpack(wqs_ref[sl, i]), _unpack(bs[i])) for i in range(7)])
        ops = []
        for h, qh in enumerate((jnp.concatenate([c11, c12], axis=1), jnp.concatenate([c21, c22], axis=1))):
            qh = (qh + k4[h * DH:(h + 1) * DH]) * qscale
            u, v, w = (qh[t * HB:(t + 1) * HB] for t in range(3))
            ops += [_ipack(u, v), _ipack(u, w), _ipack(v, w)]
        return ops

    def qk_softmax(X, h, p):
        sl = _par(p)
        xuv, xuw, xvw = X[3 * h:3 * h + 3]
        res = []
        for n in range(NN):
            c = slice(n * 128, (n + 1) * 128)
            wuw, wvw, wuv = _unpack(xuw[:, c]), _unpack(xvw[:, c]), _unpack(xuv[:, c])
            m = None
            es, ms, ls = [], [], []
            for g in range(G):
                rr = slice(g * GR // 2, (g + 1) * GR // 2)
                a = _dot(_unpack(ks_ref[sl, h, 1, rr, :]), wuw)
                bb = _dot(_unpack(ks_ref[sl, h, 2, rr, :]), wvw)
                cc = _dot(_unpack(ks_ref[sl, h, 0, rr, :]), wuv)
                sL = a + bb
                sR = cc - bb
                mg = jnp.max(_fold(jnp.maximum(sL, sR), jnp.maximum), axis=0, keepdims=True)
                m = mg if m is None else jnp.maximum(m, mg)
                parts, acc = [], None
                for sc in (sL, sR):
                    for r in range(0, GR, 32):
                        e = jnp.exp2(sc[r:r + 32] - m)
                        parts.append(_ipack(e[:16], e[16:]))
                        e8 = _fold(e, jnp.add)
                        acc = e8 if acc is None else acc + e8
                es.append(jnp.concatenate(parts, axis=0))
                ms.append(m)
                ls.append(acc)
            res.append((es, ms, ls))
        return res

    def pv(res, h, p):
        outs = []
        for n in range(NN):
            es, ms, ls = res[n]
            o, l = None, None
            for g in range(G):
                d = _dot(_unpack(vs_ref[_par(p), h, g]), _unpack(es[g]))
                if o is None:
                    o, l = d, ls[g]
                else:
                    al = jnp.exp2(ms[g - 1] - ms[g])
                    o = o * al + d
                    l = l * al + ls[g]
            outs.append(o * _recip(jnp.sum(l, axis=0, keepdims=True)))
        return outs

    def fin(oa, ob):
        def blk(x, t, n):
            return x[n][t * HB:(t + 1) * HB]
        ca = _strassen_b(blk(oa, 0, 0), blk(oa, 0, 1), blk(oa, 2, 0), blk(oa, 2, 1))
        cb = _strassen_b(blk(ob, 0, 0), blk(ob, 0, 1), blk(ob, 2, 0), blk(ob, 2, 1))
        return [_ipack(ca[i], cb[i]) for i in range(7)] + [_ipack(blk(oa, 1, n), blk(ob, 1, n)) for n in range(NN)]

    def wo_y(os, p):
        sl = _par(p)
        w1 = _unpack(wo1_ref[sl])
        mid = [_dot(w1, _unpack(os[7 + n])) for n in range(NN)]
        c11, c12, c21, c22 = _strassen_c([_dot(_unpack(wos_ref[sl, i]), _unpack(os[i])) for i in range(7)])
        return [jnp.concatenate([c11, c21], axis=0) + mid[0], jnp.concatenate([c12, c22], axis=0) + mid[1]]

    def wo(b, os, p):
        y = wo_y(os, p)
        for n in range(NN):
            acc_ref[:, cols(b, n)] += y[n]

    def epilogue(b, y):
        xs = _iunpack(xt_ref[b])
        outs = []
        for n in range(NN):
            tile = NN * b + n
            off = jnp.where(tile == tile_ref[1], S + 128, jnp.where(tile == tile_ref[0], S, tile * 128))
            hh = jnp.concatenate(_iunpack(xn_ref[:, pl.ds(pl.multiple_of(off, 128), 128)]), axis=0)
            h2 = 0.5 * hh
            g = h2 * jnp.tanh(h2) + h2
            outs.append(xs[n] + (acc_ref[:, cols(b, n)] + y[n]) * g)
        out_buf[cols(b), :] = _unpack(_ipack(outs[0], outs[1]).T)
        cp_out(b).start()

    def router_ffn():
        r = r_ref[...]
        col = lax.broadcasted_iota(I32, (1, S), 1)
        cid = (col // M) * M + 2 * (col % 128) + (col // 128) % 2
        m1 = jnp.max(r, axis=1, keepdims=True)
        i1 = jnp.min(jnp.where(r == m1, cid, S), axis=1, keepdims=True)
        r2 = jnp.where(cid == i1, -jnp.inf, r)
        m2 = jnp.max(r2, axis=1, keepdims=True)
        i2 = jnp.min(jnp.where(jnp.logical_and(r2 == m2, cid != i1), cid, S), axis=1, keepdims=True)
        tok = [jnp.min(jnp.minimum(i1, S - 1)), jnp.min(jnp.minimum(i2, S - 1))]

        def gather(sc):
            base = pl.multiple_of((sc // 16) * 16, 16)
            blk = x_buf[pl.ds(base, 16), :].astype(F32)
            sub = lax.broadcasted_iota(I32, (16, 1), 0)
            xr = jnp.sum(jnp.where(sub == sc % 16, blk, 0.0), axis=0, keepdims=True)
            mu = jnp.sum(xr, axis=1, keepdims=True) * (1.0 / D)
            xc = xr - mu
            var = jnp.sum(xc * xc, axis=1, keepdims=True) * (1.0 / D)
            return xc * lax.rsqrt(var + EPS)
        row = lax.broadcasted_iota(I32, (16, 1), 0)
        xs = jnp.where(row == 0, gather(tok[0]), jnp.where(row == 1, gather(tok[1]), 0.0)).astype(BF16)
        g = _rb(_dot(xs, wg_buf[...]))
        g = _rb(g * _sigmoid(g))
        u = _rb(_dot(xs, wu_buf[...]))
        gu = (g * u).astype(BF16)
        y = _rb(_dot(gu, wd_buf[...]))
        rs = _rb(_sigmoid(jnp.where(row == 0, m1, m2)))
        upd = _rb(y * rs)
        updt = jnp.concatenate([upd, jnp.zeros((112, D), F32)], axis=0).T
        lane = lax.broadcasted_iota(I32, (1, 128), 1)
        tiles = [NN * (t // M) + t % 2 for t in tok]
        for t in range(2):
            src_off = tiles[t] * 128
            if t == 1:
                src_off = jnp.where(tiles[1] == tiles[0], S, src_off)
            lo, hi = _iunpack(xn_ref[:, pl.ds(pl.multiple_of(src_off, 128), 128)])
            add = jnp.where(lane == (tok[t] % M) // 2, updt[:, t:t + 1], 0.0)
            xn_ref[:, S + t * 128:S + (t + 1) * 128] = _ipack(lo + add[:DL], hi + add[DL:])
            tile_ref[t] = tiles[t]

    @pl.when(j == 0)
    def _():
        w0, w1 = cp_w(0), cp_w(1)
        cp_r = pltpu.make_async_copy(wr_hbm, wr_ref, sem_r.at[0])
        cp_x(0).start(); cp_r.start(); w0[0].start()
        for i in range(1, NQ):
            cp_x(i).start()
        w0[1].start()
        acc_ref[...] = jnp.zeros(acc_ref.shape, F32)
        oc_ref[...] = jnp.zeros(oc_ref.shape, U32)
        wos_ref[1] = jnp.zeros(wos_ref.shape[1:], U32)
        wo1_ref[1] = jnp.zeros(wo1_ref.shape[1:], U32)
        cp_r.wait()
        wrc_ref[...] = jnp.broadcast_to(wr_ref[...].astype(F32).reshape(1, D), (128, D)).T
        cp_x(0).wait()
        w0[3].start(); w0[2].start()
        for c in w1:
            c.start()
        layernorm(0)
        w0[0].wait()
        stage_wq(0)
        X0 = qproj(0, 0)
        for t in range(6):
            qc_ref[t] = X0[t]
        cp_x(1).wait()
        layernorm(1)

        def ln(i, c):
            cp_x(i).wait()
            layernorm(i)
            return c
        lax.fori_loop(2, NQ, ln, 0)
        for k in range(3):
            cp_f(k).start()
        w0[1].wait()
        for h in range(2):
            for t in range(3):
                stage_k(0, h, t)
        w0[2].wait()
        stage_wo(0)
        w0[3].wait()
        stage_v(0, 0); stage_v(0, 1)

    @pl.when(j + 1 < NPAIR)
    def _():
        for c in cp_w(j + 1):
            c.wait()

    @pl.when(j + 2 < NPAIR)
    def _():
        for c in cp_w(j + 2):
            c.start()

    @pl.when(j == 1)
    def _():
        for k in range(3):
            cp_f(k).wait()
        router_ffn()

    def body(last_step):
        X = [qc_ref[t] for t in range(6)]
        o_prev = [oc_ref[t] for t in range(NO)]
        for i in range(NQ):
            last = i == NQ - 1
            if not last_step:
                if i == 3:
                    stage_v(j + 1, 0); stage_v(j + 1, 1)
                if last:
                    stage_wq(j + 1); stage_wo(j + 1)
                    for h in range(2):
                        for t in range(3):
                            stage_k(j + 1, h, t)
            ra = qk_softmax(X, 0, j)
            rb = qk_softmax(X, 1, j)
            if i == 0:
                wo(NQ - 1, o_prev, j + 1)
            elif last_step:
                epilogue(i - 1, wo_y(o_prev, j))
                if last:
                    cp_out(0).wait()
            else:
                wo(i - 1, o_prev, j)
            oa = pv(ra, 0, j)
            if not last:
                X = qproj(i + 1, j)
            elif not last_step:
                Xn = qproj(0, j + 1)
                for t in range(6):
                    qc_ref[t] = Xn[t]
            ob = pv(rb, 1, j)
            o_prev = fin(oa, ob)
        if last_step:
            epilogue(NQ - 1, wo_y(o_prev, j))
            for i in range(1, NQ):
                cp_out(i).wait()
        else:
            for t in range(NO):
                oc_ref[t] = o_prev[t]

    @pl.when(j < NPAIR - 1)
    def _():
        body(False)

    @pl.when(j == NPAIR - 1)
    def _():
        body(True)


@jax.jit
def pallas_recurrent_scan__sliding_block_cached__moe_arch_mod__prompt_kernel(
        A_x, A_k_cache, A_v_cache, A_wq, A_wo, B_x, B_w_r, B_w_gate, B_w_up, B_w_down):
    x = A_x.reshape(S, D)
    kt = jnp.swapaxes(A_k_cache, 2, 3)
    vt = jnp.swapaxes(A_v_cache, 2, 3)
    anyspec = pl.BlockSpec(memory_space=pl.ANY)
    out = pl.pallas_call(
        _kernel,
        grid=(NPAIR,),
        in_specs=[anyspec] * 9,
        out_specs=anyspec,
        out_shape=jax.ShapeDtypeStruct((S, D), BF16),
        scratch_shapes=[
            pltpu.VMEM((S, D), BF16),
            pltpu.VMEM((NQ, D, 128), U32),
            pltpu.VMEM((DL, S + 256), U32),
            pltpu.VMEM((NQ, 5, 128, 128), U32),
            pltpu.VMEM((D, S), F32),
            pltpu.VMEM((2, D, PW), BF16),
            pltpu.VMEM((2, PW, D), BF16),
            pltpu.VMEM((2, 2, DH, W), BF16),
            pltpu.VMEM((2, 2, DH, W), BF16),
            pltpu.VMEM((2, 7, DH // 2, 256), U32),
            pltpu.VMEM((2, PW // 2, 128), U32),
            pltpu.VMEM((2, 2, 3, KH // 2, 128), U32),
            pltpu.VMEM((2, 2, G, DH // 2, 128), U32),
            pltpu.VMEM((2, 7, DL // 2, 128), U32),
            pltpu.VMEM((2, DL, 128), U32),
            pltpu.VMEM((6, HB, M), U32),
            pltpu.VMEM((NO, HB, 128), U32),
            pltpu.VMEM((1, S), F32),
            pltpu.SMEM((2,), I32),
            pltpu.VMEM((D, FF), BF16),
            pltpu.VMEM((D, FF), BF16),
            pltpu.VMEM((FF, D), BF16),
            pltpu.VMEM((S, D), BF16),
            pltpu.VMEM((KH, 128), F32),
            pltpu.VMEM((D, 128), F32),
            pltpu.VMEM((D,), BF16),
            pltpu.SemaphoreType.DMA((NQ,)),
            pltpu.SemaphoreType.DMA((8,)),
            pltpu.SemaphoreType.DMA((3,)),
            pltpu.SemaphoreType.DMA((NQ,)),
            pltpu.SemaphoreType.DMA((1,)),
        ],
        compiler_params=pltpu.CompilerParams(
            dimension_semantics=("arbitrary",),
            vmem_limit_bytes=100 * 1024 * 1024,
            disable_bounds_checks=True),
        name="fused_attn_mod",
    )(x, kt, vt, A_wq, A_wo, B_w_r, B_w_gate, B_w_up, B_w_down)
    return out.reshape(1, S, D)
```

```python
import jax
import jax.numpy as jnp
from jax import lax
from jax.experimental import pallas as pl
from jax.experimental.pallas import tpu as pltpu

F32 = jnp.float32
BF16 = jnp.bfloat16
U32 = jnp.uint32
I32 = jnp.int32
LOG2E = 1.4426950408889634

S, D = 2048, 640
H, DH, W = 32, 192, 512
FF = 1536
EPS = 1.0013580322265625e-05
HB = 64
KH = W // 2
PW = 2 * DH
NPAIR = H // 2
M = 256
NQ = S // M
NN = M // 128
DL = D // 2
G = 4
GR = KH // G
NO = 9


def _pack(x):
    return pltpu.bitcast(x, U32)


def _unpack(x):
    return pltpu.bitcast(x, BF16)


def _bf(x):
    parts = [pltpu.bitcast(x[:, i * 128:(i + 1) * 128].astype(BF16), U32) for i in range(x.shape[1] // 128)]
    return pltpu.bitcast(jnp.concatenate(parts, axis=1), BF16)


def _ipack(a, b):
    return pltpu.pack_elementwise([a, b], packed_dtype=BF16)


def _iunpack(u):
    return (pltpu.unpack_elementwise(u, index=0, packed_dtype=BF16, unpacked_dtype=F32),
            pltpu.unpack_elementwise(u, index=1, packed_dtype=BF16, unpacked_dtype=F32))


def _interleave(a, b):
    return _unpack(_ipack(a, b)).astype(F32)


def _par(p):
    return p & 1


def _sigmoid(x):
    return 0.5 * jnp.tanh(0.5 * x) + 0.5


def _rb(x):
    return x.astype(BF16).astype(F32)


def _inv_std(var):
    return 1.0 / _rb(jnp.sqrt(_rb(_rb(var) + EPS)))


def _recip(l):
    r = pl.reciprocal(l, approx=True)
    return r * (2.0 - l * r)


def _dot(a, b):
    return jnp.dot(a, b, preferred_element_type=F32)


def _fold(x, op):
    parts = [x[i:i + 8] for i in range(0, x.shape[0], 8)]
    while len(parts) > 1:
        nxt = [op(parts[i], parts[i + 1]) for i in range(0, len(parts) - 1, 2)]
        if len(parts) % 2:
            nxt.append(parts[-1])
        parts = nxt
    return parts[0]


def _strassen_a(a11, a12, a21, a22):
    return [a11 + a22, a21 + a22, a11, a22, a11 + a12, a21 - a11, a12 - a22]


def _strassen_b(b11, b12, b21, b22):
    return [b11 + b22, b11, b12 - b22, b21 - b11, b22, b11 + b12, b21 + b22]


def _strassen_c(m):
    m1, m2, m3, m4, m5, m6, m7 = m
    return m1 + m4 - m5 + m7, m3 + m5, m2 + m4, m1 - m2 + m3 + m6


def _kernel(x_hbm, kt_hbm, vt_hbm, wq_hbm, wo_hbm, wr_hbm, wg_hbm, wu_hbm, wd_hbm,
            out_hbm,
            x_buf, xt_ref, xn_ref, sx_ref, acc_ref, wq_buf, wo_buf, kt_buf, vt_buf,
            wqs_ref, wq4_ref, ks_ref, vs_ref, wos_ref, wo1_ref, qc_ref, oc_ref, r_ref, tile_ref,
            wg_buf, wu_buf, wd_buf, out_buf, tmp_ref, wrc_ref, wr_ref,
            sem_x, sem_w, sem_f, sem_o, sem_r):
    j = pl.program_id(0)
    sk = kt_hbm.shape[3]
    qscale = (DH ** -0.5) * LOG2E

    def cp_x(i):
        return pltpu.make_async_copy(x_hbm.at[cols(i), :], x_buf.at[cols(i), :], sem_x.at[i])

    def cp_w(p):
        sl = _par(p)
        off = p * PW if isinstance(p, int) else pl.multiple_of(p * PW, 128)
        return [
            pltpu.make_async_copy(wq_hbm.at[:, pl.ds(off, PW)], wq_buf.at[sl], sem_w.at[sl]),
            pltpu.make_async_copy(kt_hbm.at[0, pl.ds(2 * p, 2), :, pl.ds(sk - W, W)], kt_buf.at[sl], sem_w.at[2 + sl]),
            pltpu.make_async_copy(wo_hbm.at[pl.ds(off, PW), :], wo_buf.at[sl], sem_w.at[6 + sl]),
            pltpu.make_async_copy(vt_hbm.at[0, pl.ds(2 * p, 2), :, pl.ds(sk - W, W)], vt_buf.at[sl], sem_w.at[4 + sl]),
        ]

    def cp_f(k):
        src, dst = [(wg_hbm, wg_buf), (wu_hbm, wu_buf), (wd_hbm, wd_buf)][k]
        return pltpu.make_async_copy(src, dst, sem_f.at[k])

    def cp_out(i):
        return pltpu.make_async_copy(out_buf.at[cols(i), :], out_hbm.at[cols(i), :], sem_o.at[i])

    def cols(b, n=None):
        off, sz = (b * M, M) if n is None else (b * M + n * 128, 128)
        return pl.ds(off if isinstance(b, int) else pl.multiple_of(off, 128), sz)

    def layernorm(b):
        xt = _pack(x_buf[cols(b), :]).T
        xt_ref[b] = xt
        piv = _iunpack(xt[0:1])
        s1, s2 = [[None] * 4, [None] * 4], [[None] * 4, [None] * 4]
        for g in range(D // 8):
            for n, x in enumerate(_iunpack(xt[g * 8:(g + 1) * 8])):
                xs = x - piv[n]
                a = g % 4
                s1[n][a] = xs if s1[n][a] is None else s1[n][a] + xs
                s2[n][a] = xs * xs if s2[n][a] is None else s2[n][a] + xs * xs
        mean, rstd = [], []
        for n in range(2):
            m1 = jnp.sum((s1[n][0] + s1[n][1]) + (s1[n][2] + s1[n][3]), axis=0, keepdims=True) * (1.0 / D)
            m2 = jnp.sum((s2[n][0] + s2[n][1]) + (s2[n][2] + s2[n][3]), axis=0, keepdims=True) * (1.0 / D)
            mean.append(_rb(piv[n] + m1))
            rstd.append(_inv_std(jnp.maximum(m2 - m1 * m1, 0.0)))
        b2 = b if isinstance(b, int) else (b + NQ) % NQ
        racc = [None, None]

        def norm_group(g):
            xl = _iunpack(xt_ref[b2, g * 8:(g + 1) * 8, :])
            xh = _iunpack(xt_ref[b2, DL + g * 8:DL + (g + 1) * 8, :])
            res = []
            for n in range(2):
                dl, dh = _iunpack(_ipack(xl[n] - mean[n], xh[n] - mean[n]))
                u = _ipack(dl * rstd[n], dh * rstd[n])
                xn_ref[g * 8:(g + 1) * 8, cols(b, n)] = u
                lo, hi = _iunpack(u)
                t = lo * wrc_ref[g * 8:(g + 1) * 8, :] + hi * wrc_ref[DL + g * 8:DL + (g + 1) * 8, :]
                racc[n] = t if racc[n] is None else racc[n] + t
                res.append((lo, hi))
            return res
        for g in range(16):
            top, bot = norm_group(g), norm_group(g + 16)
            cs = [_strassen_b(top[0][i], top[1][i], bot[0][i], bot[1][i]) for i in range(2)]
            for t, i in enumerate((0, 2, 3, 5, 6)):
                sx_ref[b, t, g * 8:(g + 1) * 8, :] = _ipack(cs[0][i], cs[1][i])
        for g in range(32, DL // 8):
            norm_group(g)
        for n in range(2):
            r_ref[:, cols(b, n)] = _rb(jnp.sum(racc[n], axis=0, keepdims=True))

    def stage_wq(p):
        sl = _par(p)
        w = wq_buf[sl].astype(F32)
        wt = _interleave(w[:DL], w[DL:]).T
        a = _strassen_a(wt[:DH, :256], wt[:DH, 256:512], wt[DH:, :256], wt[DH:, 256:512])
        for i in range(7):
            wqs_ref[sl, i] = _pack(_bf(a[i]))
        wq4_ref[sl] = _pack(_bf(wt[:, 512:]))

    def stage_k(p, h, t):
        sl = _par(p)

        def blk(b, half):
            return kt_buf[sl, h, b * HB:(b + 1) * HB, half * KH:(half + 1) * KH].astype(F32)
        top, bot = [lambda: (blk(0, 1), blk(1, 0) + blk(1, 1)),
                    lambda: (blk(0, 0), blk(2, 0) + blk(2, 1)),
                    lambda: (blk(1, 0), -blk(2, 1))][t]()
        tmp_ref[...] = _interleave(top, bot).T
        for c in range(KH // 32):
            ld = [tmp_ref[pl.ds(c * 32 + o, 8, stride=4), :] for o in range(4)]
            ks_ref[sl, h, t, c * 16:(c + 1) * 16, :] = _ipack(
                jnp.concatenate(ld[:2], axis=0), jnp.concatenate(ld[2:], axis=0))

    def stage_v(p, h):
        v = _pack(vt_buf[_par(p), h])
        for g in range(G):
            vs_ref[_par(p), h, g] = jnp.concatenate(
                [v[:, g * GR:(g + 1) * GR], v[:, KH + g * GR:KH + (g + 1) * GR]], axis=1)

    def stage_wo(p):
        sl = _par(p)
        w = wo_buf[sl].astype(F32)
        wt = _interleave(w[:DH], w[DH:]).T
        wo1_ref[sl] = _pack(wt[:, 128:256].astype(BF16))
        a = _strassen_a(wt[:DL, :128], wt[:DL, 256:], wt[DL:, :128], wt[DL:, 256:])
        for i in range(7):
            wos_ref[sl, i] = _pack(a[i].astype(BF16))

    def qproj(b, p):
        sl = _par(p)
        xn = xn_ref[:, cols(b)]
        k4 = _dot(_unpack(wq4_ref[sl]), _unpack(xn[256:]))
        bs = [sx_ref[b, 0], xn[:128, :128], sx_ref[b, 1], sx_ref[b, 2], xn[128:256, 128:], sx_ref[b, 3], sx_ref[b, 4]]
        c11, c12, c21, c22 = _strassen_c([_dot(_unpack(wqs_ref[sl, i]), _unpack(bs[i])) for i in range(7)])
        ops = []
        for h, qh in enumerate((jnp.concatenate([c11, c12], axis=1), jnp.concatenate([c21, c22], axis=1))):
            qh = (qh + k4[h * DH:(h + 1) * DH]) * qscale
            u, v, w = (qh[t * HB:(t + 1) * HB] for t in range(3))
            ops += [_ipack(u, v), _ipack(u, w), _ipack(v, w)]
        return ops

    def qk_softmax(X, h, p):
        sl = _par(p)
        xuv, xuw, xvw = X[3 * h:3 * h + 3]
        res = []
        for n in range(NN):
            c = slice(n * 128, (n + 1) * 128)
            wuw, wvw, wuv = _unpack(xuw[:, c]), _unpack(xvw[:, c]), _unpack(xuv[:, c])
            m = None
            es, ms, ls = [], [], []
            for g in range(G):
                rr = slice(g * GR // 2, (g + 1) * GR // 2)
                a = _dot(_unpack(ks_ref[sl, h, 1, rr, :]), wuw)
                bb = _dot(_unpack(ks_ref[sl, h, 2, rr, :]), wvw)
                cc = _dot(_unpack(ks_ref[sl, h, 0, rr, :]), wuv)
                sL = a + bb
                sR = cc - bb
                mg = jnp.max(_fold(jnp.maximum(sL, sR), jnp.maximum), axis=0, keepdims=True)
                m = mg if m is None else jnp.maximum(m, mg)
                parts, acc = [], None
                for sc in (sL, sR):
                    for r in range(0, GR, 32):
                        e = jnp.exp2(sc[r:r + 32] - m)
                        parts.append(_ipack(e[:16], e[16:]))
                        e8 = _fold(e, jnp.add)
                        acc = e8 if acc is None else acc + e8
                es.append(jnp.concatenate(parts, axis=0))
                ms.append(m)
                ls.append(acc)
            res.append((es, ms, ls))
        return res

    def pv(res, h, p):
        outs = []
        for n in range(NN):
            es, ms, ls = res[n]
            o, l = None, None
            for g in range(G):
                d = _dot(_unpack(vs_ref[_par(p), h, g]), _unpack(es[g]))
                if o is None:
                    o, l = d, ls[g]
                else:
                    al = jnp.exp2(ms[g - 1] - ms[g])
                    o = o * al + d
                    l = l * al + ls[g]
            outs.append(o * _recip(jnp.sum(l, axis=0, keepdims=True)))
        return outs

    def fin(oa, ob):
        def blk(x, t, n):
            return x[n][t * HB:(t + 1) * HB]
        ca = _strassen_b(blk(oa, 0, 0), blk(oa, 0, 1), blk(oa, 2, 0), blk(oa, 2, 1))
        cb = _strassen_b(blk(ob, 0, 0), blk(ob, 0, 1), blk(ob, 2, 0), blk(ob, 2, 1))
        return [_ipack(ca[i], cb[i]) for i in range(7)] + [_ipack(blk(oa, 1, n), blk(ob, 1, n)) for n in range(NN)]

    def wo_y(os, p):
        sl = _par(p)
        w1 = _unpack(wo1_ref[sl])
        mid = [_dot(w1, _unpack(os[7 + n])) for n in range(NN)]
        c11, c12, c21, c22 = _strassen_c([_dot(_unpack(wos_ref[sl, i]), _unpack(os[i])) for i in range(7)])
        return [jnp.concatenate([c11, c21], axis=0) + mid[0], jnp.concatenate([c12, c22], axis=0) + mid[1]]

    def wo(b, os, p):
        y = wo_y(os, p)
        for n in range(NN):
            acc_ref[:, cols(b, n)] += y[n]

    def epilogue(b, y):
        xs = _iunpack(xt_ref[b])
        outs = []
        for n in range(NN):
            tile = NN * b + n
            off = jnp.where(tile == tile_ref[1], S + 128, jnp.where(tile == tile_ref[0], S, tile * 128))
            hh = jnp.concatenate(_iunpack(xn_ref[:, pl.ds(pl.multiple_of(off, 128), 128)]), axis=0)
            h2 = 0.5 * hh
            g = h2 * jnp.tanh(h2) + h2
            outs.append(xs[n] + (acc_ref[:, cols(b, n)] + y[n]) * g)
        out_buf[cols(b), :] = _unpack(_ipack(outs[0], outs[1]).T)
        cp_out(b).start()

    def router_ffn():
        r = r_ref[...]
        col = lax.broadcasted_iota(I32, (1, S), 1)
        cid = (col // M) * M + 2 * (col % 128) + (col // 128) % 2
        m1 = jnp.max(r, axis=1, keepdims=True)
        i1 = jnp.min(jnp.where(r == m1, cid, S), axis=1, keepdims=True)
        r2 = jnp.where(cid == i1, -jnp.inf, r)
        m2 = jnp.max(r2, axis=1, keepdims=True)
        i2 = jnp.min(jnp.where(jnp.logical_and(r2 == m2, cid != i1), cid, S), axis=1, keepdims=True)
        tok = [jnp.min(jnp.minimum(i1, S - 1)), jnp.min(jnp.minimum(i2, S - 1))]

        def gather(sc):
            base = pl.multiple_of((sc // 16) * 16, 16)
            blk = x_buf[pl.ds(base, 16), :].astype(F32)
            sub = lax.broadcasted_iota(I32, (16, 1), 0)
            xr = jnp.sum(jnp.where(sub == sc % 16, blk, 0.0), axis=0, keepdims=True)
            mu = jnp.sum(xr, axis=1, keepdims=True) * (1.0 / D)
            xc = xr - mu
            var = jnp.sum(xc * xc, axis=1, keepdims=True) * (1.0 / D)
            return _rb(xr - _rb(mu)) * _inv_std(var)
        row = lax.broadcasted_iota(I32, (16, 1), 0)
        xs = jnp.where(row == 0, gather(tok[0]), jnp.where(row == 1, gather(tok[1]), 0.0)).astype(BF16)
        g = _rb(_dot(xs, wg_buf[...]))
        g = _rb(g * _sigmoid(g))
        u = _rb(_dot(xs, wu_buf[...]))
        gu = (g * u).astype(BF16)
        y = _rb(_dot(gu, wd_buf[...]))
        rs = _rb(_sigmoid(jnp.where(row == 0, m1, m2)))
        upd = _rb(y * rs)
        updt = jnp.concatenate([upd, jnp.zeros((112, D), F32)], axis=0).T
        lane = lax.broadcasted_iota(I32, (1, 128), 1)
        tiles = [NN * (t // M) + t % 2 for t in tok]
        for t in range(2):
            src_off = tiles[t] * 128
            if t == 1:
                src_off = jnp.where(tiles[1] == tiles[0], S, src_off)
            lo, hi = _iunpack(xn_ref[:, pl.ds(pl.multiple_of(src_off, 128), 128)])
            add = jnp.where(lane == (tok[t] % M) // 2, updt[:, t:t + 1], 0.0)
            xn_ref[:, S + t * 128:S + (t + 1) * 128] = _ipack(lo + add[:DL], hi + add[DL:])
            tile_ref[t] = tiles[t]

    @pl.when(j == 0)
    def _():
        w0, w1 = cp_w(0), cp_w(1)
        cp_r = pltpu.make_async_copy(wr_hbm, wr_ref, sem_r.at[0])
        cp_x(0).start(); cp_r.start(); w0[0].start()
        for i in range(1, NQ):
            cp_x(i).start()
        w0[1].start()
        acc_ref[...] = jnp.zeros(acc_ref.shape, F32)
        oc_ref[...] = jnp.zeros(oc_ref.shape, U32)
        wos_ref[1] = jnp.zeros(wos_ref.shape[1:], U32)
        wo1_ref[1] = jnp.zeros(wo1_ref.shape[1:], U32)
        cp_r.wait()
        wrc_ref[...] = jnp.broadcast_to(wr_ref[...].astype(F32).reshape(1, D), (128, D)).T
        cp_x(0).wait()
        w0[3].start(); w0[2].start()
        for c in w1:
            c.start()
        layernorm(0)
        w0[0].wait()
        stage_wq(0)
        X0 = qproj(0, 0)
        for t in range(6):
            qc_ref[t] = X0[t]
        cp_x(1).wait()
        layernorm(1)

        def ln(i, c):
            cp_x(i).wait()
            layernorm(i)
            return c
        lax.fori_loop(2, NQ, ln, 0)
        for k in range(3):
            cp_f(k).start()
        w0[1].wait()
        for h in range(2):
            for t in range(3):
                stage_k(0, h, t)
        w0[2].wait()
        stage_wo(0)
        w0[3].wait()
        stage_v(0, 0); stage_v(0, 1)

    @pl.when(j + 1 < NPAIR)
    def _():
        for c in cp_w(j + 1):
            c.wait()

    @pl.when(j + 2 < NPAIR)
    def _():
        for c in cp_w(j + 2):
            c.start()

    @pl.when(j == 1)
    def _():
        for k in range(3):
            cp_f(k).wait()
        router_ffn()

    def body(last_step):
        X = [qc_ref[t] for t in range(6)]
        o_prev = [oc_ref[t] for t in range(NO)]
        for i in range(NQ):
            last = i == NQ - 1
            if not last_step:
                if i == 3:
                    stage_v(j + 1, 0); stage_v(j + 1, 1)
                if last:
                    stage_wq(j + 1); stage_wo(j + 1)
                    for h in range(2):
                        for t in range(3):
                            stage_k(j + 1, h, t)
            ra = qk_softmax(X, 0, j)
            rb = qk_softmax(X, 1, j)
            if i == 0:
                wo(NQ - 1, o_prev, j + 1)
            elif last_step:
                epilogue(i - 1, wo_y(o_prev, j))
                if last:
                    cp_out(0).wait()
            else:
                wo(i - 1, o_prev, j)
            oa = pv(ra, 0, j)
            if not last:
                X = qproj(i + 1, j)
            elif not last_step:
                Xn = qproj(0, j + 1)
                for t in range(6):
                    qc_ref[t] = Xn[t]
            ob = pv(rb, 1, j)
            o_prev = fin(oa, ob)
        if last_step:
            epilogue(NQ - 1, wo_y(o_prev, j))
            for i in range(1, NQ):
                cp_out(i).wait()
        else:
            for t in range(NO):
                oc_ref[t] = o_prev[t]

    @pl.when(j < NPAIR - 1)
    def _():
        body(False)

    @pl.when(j == NPAIR - 1)
    def _():
        body(True)


@jax.jit
def pallas_recurrent_scan__sliding_block_cached__moe_arch_mod__prompt_kernel(
        A_x, A_k_cache, A_v_cache, A_wq, A_wo, B_x, B_w_r, B_w_gate, B_w_up, B_w_down):
    x = A_x.reshape(S, D)
    kt = jnp.swapaxes(A_k_cache, 2, 3)
    vt = jnp.swapaxes(A_v_cache, 2, 3)
    anyspec = pl.BlockSpec(memory_space=pl.ANY)
    out = pl.pallas_call(
        _kernel,
        grid=(NPAIR,),
        in_specs=[anyspec] * 9,
        out_specs=anyspec,
        out_shape=jax.ShapeDtypeStruct((S, D), BF16),
        scratch_shapes=[
            pltpu.VMEM((S, D), BF16),
            pltpu.VMEM((NQ, D, 128), U32),
            pltpu.VMEM((DL, S + 256), U32),
            pltpu.VMEM((NQ, 5, 128, 128), U32),
            pltpu.VMEM((D, S), F32),
            pltpu.VMEM((2, D, PW), BF16),
            pltpu.VMEM((2, PW, D), BF16),
            pltpu.VMEM((2, 2, DH, W), BF16),
            pltpu.VMEM((2, 2, DH, W), BF16),
            pltpu.VMEM((2, 7, DH // 2, 256), U32),
            pltpu.VMEM((2, PW // 2, 128), U32),
            pltpu.VMEM((2, 2, 3, KH // 2, 128), U32),
            pltpu.VMEM((2, 2, G, DH // 2, 128), U32),
            pltpu.VMEM((2, 7, DL // 2, 128), U32),
            pltpu.VMEM((2, DL, 128), U32),
            pltpu.VMEM((6, HB, M), U32),
            pltpu.VMEM((NO, HB, 128), U32),
            pltpu.VMEM((1, S), F32),
            pltpu.SMEM((2,), I32),
            pltpu.VMEM((D, FF), BF16),
            pltpu.VMEM((D, FF), BF16),
            pltpu.VMEM((FF, D), BF16),
            pltpu.VMEM((S, D), BF16),
            pltpu.VMEM((KH, 128), F32),
            pltpu.VMEM((D, 128), F32),
            pltpu.VMEM((D,), BF16),
            pltpu.SemaphoreType.DMA((NQ,)),
            pltpu.SemaphoreType.DMA((8,)),
            pltpu.SemaphoreType.DMA((3,)),
            pltpu.SemaphoreType.DMA((NQ,)),
            pltpu.SemaphoreType.DMA((1,)),
        ],
        compiler_params=pltpu.CompilerParams(
            dimension_semantics=("arbitrary",),
            vmem_limit_bytes=100 * 1024 * 1024,
            disable_bounds_checks=True),
        name="fused_attn_mod",
    )(x, kt, vt, A_wq, A_wo, B_w_r, B_w_gate, B_w_up, B_w_down)
    return out.reshape(1, S, D)
```

```python
import jax
import jax.numpy as jnp
from jax import lax
from jax.experimental import pallas as pl
from jax.experimental.pallas import tpu as pltpu

F32 = jnp.float32
BF16 = jnp.bfloat16
U32 = jnp.uint32
I32 = jnp.int32
LOG2E = 1.4426950408889634

S, D = 2048, 640
H, DH, W = 32, 192, 512
FF = 1536
EPS = 1.0013580322265625e-05
HB = 64
KH = W // 2
PW = 2 * DH
NPAIR = H // 2
M = 256
NQ = S // M
NN = M // 128
DL = D // 2
G = 4
GR = KH // G
NO = 9


def _pack(x):
    return pltpu.bitcast(x, U32)


def _unpack(x):
    return pltpu.bitcast(x, BF16)


def _bf(x):
    parts = [pltpu.bitcast(x[:, i * 128:(i + 1) * 128].astype(BF16), U32) for i in range(x.shape[1] // 128)]
    return pltpu.bitcast(jnp.concatenate(parts, axis=1), BF16)


def _ipack(a, b):
    return pltpu.pack_elementwise([a, b], packed_dtype=BF16)


def _iunpack(u):
    return (pltpu.unpack_elementwise(u, index=0, packed_dtype=BF16, unpacked_dtype=F32),
            pltpu.unpack_elementwise(u, index=1, packed_dtype=BF16, unpacked_dtype=F32))


def _interleave(a, b):
    return _unpack(_ipack(a, b)).astype(F32)


def _par(p):
    return p & 1


def _sigmoid(x):
    return 0.5 * jnp.tanh(0.5 * x) + 0.5


def _rb(x):
    return x.astype(BF16).astype(F32)


def _inv_std(var):
    return 1.0 / _rb(jnp.sqrt(_rb(_rb(var) + EPS)))


def _recip(l):
    r = pl.reciprocal(l, approx=True)
    return r * (2.0 - l * r)


def _dot(a, b):
    return jnp.dot(a, b, preferred_element_type=F32)


def _fold(x, op):
    parts = [x[i:i + 8] for i in range(0, x.shape[0], 8)]
    while len(parts) > 1:
        nxt = [op(parts[i], parts[i + 1]) for i in range(0, len(parts) - 1, 2)]
        if len(parts) % 2:
            nxt.append(parts[-1])
        parts = nxt
    return parts[0]


def _strassen_a(a11, a12, a21, a22):
    return [a11 + a22, a21 + a22, a11, a22, a11 + a12, a21 - a11, a12 - a22]


def _strassen_b(b11, b12, b21, b22):
    return [b11 + b22, b11, b12 - b22, b21 - b11, b22, b11 + b12, b21 + b22]


def _strassen_c(m):
    m1, m2, m3, m4, m5, m6, m7 = m
    return m1 + m4 - m5 + m7, m3 + m5, m2 + m4, m1 - m2 + m3 + m6


def _kernel(x_hbm, kt_hbm, vt_hbm, wq_hbm, wo_hbm, wr_hbm, wg_hbm, wu_hbm, wd_hbm,
            out_hbm,
            x_buf, xt_ref, xn_ref, sx_ref, acc_ref, wq_buf, wo_buf, kt_buf, vt_buf,
            wqs_ref, wq4_ref, ks_ref, vs_ref, wos_ref, wo1_ref, qc_ref, oc_ref, r_ref, tile_ref,
            wg_buf, wu_buf, wd_buf, out_buf, tmp_ref, wrc_ref, wr_ref,
            sem_x, sem_w, sem_f, sem_o, sem_r):
    j = pl.program_id(0)
    sk = kt_hbm.shape[3]
    qscale = (DH ** -0.5) * LOG2E

    def cp_x(i):
        return pltpu.make_async_copy(x_hbm.at[cols(i), :], x_buf.at[cols(i), :], sem_x.at[i])

    def cp_w(p):
        sl = _par(p)
        off = p * PW if isinstance(p, int) else pl.multiple_of(p * PW, 128)
        return [
            pltpu.make_async_copy(wq_hbm.at[:, pl.ds(off, PW)], wq_buf.at[sl], sem_w.at[sl]),
            pltpu.make_async_copy(kt_hbm.at[0, pl.ds(2 * p, 2), :, pl.ds(sk - W, W)], kt_buf.at[sl], sem_w.at[2 + sl]),
            pltpu.make_async_copy(wo_hbm.at[pl.ds(off, PW), :], wo_buf.at[sl], sem_w.at[6 + sl]),
            pltpu.make_async_copy(vt_hbm.at[0, pl.ds(2 * p, 2), :, pl.ds(sk - W, W)], vt_buf.at[sl], sem_w.at[4 + sl]),
        ]

    def cp_f(k):
        src, dst = [(wg_hbm, wg_buf), (wu_hbm, wu_buf), (wd_hbm, wd_buf)][k]
        return pltpu.make_async_copy(src, dst, sem_f.at[k])

    def cp_out(i):
        return pltpu.make_async_copy(out_buf.at[cols(i), :], out_hbm.at[cols(i), :], sem_o.at[i])

    def cols(b, n=None):
        off, sz = (b * M, M) if n is None else (b * M + n * 128, 128)
        return pl.ds(off if isinstance(b, int) else pl.multiple_of(off, 128), sz)

    def layernorm(b):
        xt = _pack(x_buf[cols(b), :]).T
        xt_ref[b] = xt
        piv = _iunpack(xt[0:1])
        s1, s2 = [[None] * 4, [None] * 4], [[None] * 4, [None] * 4]
        for g in range(D // 8):
            for n, x in enumerate(_iunpack(xt[g * 8:(g + 1) * 8])):
                xs = x - piv[n]
                a = g % 4
                s1[n][a] = xs if s1[n][a] is None else s1[n][a] + xs
                s2[n][a] = xs * xs if s2[n][a] is None else s2[n][a] + xs * xs
        mean, rstd = [], []
        for n in range(2):
            m1 = jnp.sum((s1[n][0] + s1[n][1]) + (s1[n][2] + s1[n][3]), axis=0, keepdims=True) * (1.0 / D)
            m2 = jnp.sum((s2[n][0] + s2[n][1]) + (s2[n][2] + s2[n][3]), axis=0, keepdims=True) * (1.0 / D)
            mean.append(_rb(piv[n] + m1))
            rstd.append(_inv_std(jnp.maximum(m2 - m1 * m1, 0.0)))
        b2 = b if isinstance(b, int) else (b + NQ) % NQ
        racc = [None, None]

        def norm_group(g):
            xl = _iunpack(xt_ref[b2, g * 8:(g + 1) * 8, :])
            xh = _iunpack(xt_ref[b2, DL + g * 8:DL + (g + 1) * 8, :])
            res = []
            for n in range(2):
                dl, dh = _iunpack(_ipack(xl[n] - mean[n], xh[n] - mean[n]))
                u = _ipack(dl * rstd[n], dh * rstd[n])
                xn_ref[g * 8:(g + 1) * 8, cols(b, n)] = u
                lo, hi = _iunpack(u)
                t = lo * wrc_ref[g * 8:(g + 1) * 8, :] + hi * wrc_ref[DL + g * 8:DL + (g + 1) * 8, :]
                racc[n] = t if racc[n] is None else racc[n] + t
                res.append((lo, hi))
            return res
        for g in range(16):
            top, bot = norm_group(g), norm_group(g + 16)
            cs = [_strassen_b(top[0][i], top[1][i], bot[0][i], bot[1][i]) for i in range(2)]
            for t, i in enumerate((0, 2, 3, 5, 6)):
                sx_ref[b, t, g * 8:(g + 1) * 8, :] = _ipack(cs[0][i], cs[1][i])
        for g in range(32, DL // 8):
            norm_group(g)
        for n in range(2):
            r_ref[:, cols(b, n)] = _rb(jnp.sum(racc[n], axis=0, keepdims=True))

    def stage_wq(p):
        sl = _par(p)
        w = wq_buf[sl].astype(F32)
        wt = _interleave(w[:DL], w[DL:]).T
        a = _strassen_a(wt[:DH, :256], wt[:DH, 256:512], wt[DH:, :256], wt[DH:, 256:512])
        for i in range(7):
            wqs_ref[sl, i] = _pack(_bf(a[i]))
        wq4_ref[sl] = _pack(_bf(wt[:, 512:]))

    def stage_k(p, h, t):
        sl = _par(p)

        def blk(b, half):
            return kt_buf[sl, h, b * HB:(b + 1) * HB, half * KH:(half + 1) * KH].astype(F32)
        top, bot = [lambda: (blk(0, 1), blk(1, 0) + blk(1, 1)),
                    lambda: (blk(0, 0), blk(2, 0) + blk(2, 1)),
                    lambda: (blk(1, 0), -blk(2, 1))][t]()
        tmp_ref[...] = _interleave(top, bot).T
        for c in range(KH // 32):
            ld = [tmp_ref[pl.ds(c * 32 + o, 8, stride=4), :] for o in range(4)]
            ks_ref[sl, h, t, c * 16:(c + 1) * 16, :] = _ipack(
                jnp.concatenate(ld[:2], axis=0), jnp.concatenate(ld[2:], axis=0))

    def stage_v(p, h):
        v = _pack(vt_buf[_par(p), h])
        for g in range(G):
            vs_ref[_par(p), h, g] = jnp.concatenate(
                [v[:, g * GR:(g + 1) * GR], v[:, KH + g * GR:KH + (g + 1) * GR]], axis=1)

    def stage_wo(p):
        sl = _par(p)
        w = wo_buf[sl].astype(F32)
        wt = _interleave(w[:DH], w[DH:]).T
        wo1_ref[sl] = _pack(wt[:, 128:256].astype(BF16))
        a = _strassen_a(wt[:DL, :128], wt[:DL, 256:], wt[DL:, :128], wt[DL:, 256:])
        for i in range(7):
            wos_ref[sl, i] = _pack(a[i].astype(BF16))

    def qproj(b, p):
        sl = _par(p)
        xn = xn_ref[:, cols(b)]
        k4 = _dot(_unpack(wq4_ref[sl]), _unpack(xn[256:]))
        bs = [sx_ref[b, 0], xn[:128, :128], sx_ref[b, 1], sx_ref[b, 2], xn[128:256, 128:], sx_ref[b, 3], sx_ref[b, 4]]
        c11, c12, c21, c22 = _strassen_c([_dot(_unpack(wqs_ref[sl, i]), _unpack(bs[i])) for i in range(7)])
        ops = []
        for h, qh in enumerate((jnp.concatenate([c11, c12], axis=1), jnp.concatenate([c21, c22], axis=1))):
            qh = (qh + k4[h * DH:(h + 1) * DH]) * qscale
            u, v, w = (qh[t * HB:(t + 1) * HB] for t in range(3))
            ops += [_ipack(u, v), _ipack(u, w), _ipack(v, w)]
        return ops

    def qk_softmax(X, h, p):
        sl = _par(p)
        xuv, xuw, xvw = X[3 * h:3 * h + 3]
        res = []
        for n in range(NN):
            c = slice(n * 128, (n + 1) * 128)
            wuw, wvw, wuv = _unpack(xuw[:, c]), _unpack(xvw[:, c]), _unpack(xuv[:, c])
            m = None
            es, ms, ls = [], [], []
            for g in range(G):
                rr = slice(g * GR // 2, (g + 1) * GR // 2)
                a = _dot(_unpack(ks_ref[sl, h, 1, rr, :]), wuw)
                bb = _dot(_unpack(ks_ref[sl, h, 2, rr, :]), wvw)
                cc = _dot(_unpack(ks_ref[sl, h, 0, rr, :]), wuv)
                sL = a + bb
                sR = cc - bb
                mg = jnp.max(_fold(jnp.maximum(sL, sR), jnp.maximum), axis=0, keepdims=True)
                m = mg if m is None else jnp.maximum(m, mg)
                parts, acc = [], None
                for sc in (sL, sR):
                    for r in range(0, GR, 32):
                        e = jnp.exp2(sc[r:r + 32] - m)
                        parts.append(_ipack(e[:16], e[16:]))
                        e8 = _fold(e, jnp.add)
                        acc = e8 if acc is None else acc + e8
                es.append(jnp.concatenate(parts, axis=0))
                ms.append(m)
                ls.append(acc)
            res.append((es, ms, ls))
        return res

    def pv(res, h, p):
        outs = []
        for n in range(NN):
            es, ms, ls = res[n]
            o, l = None, None
            for g in range(G):
                d = _dot(_unpack(vs_ref[_par(p), h, g]), _unpack(es[g]))
                if o is None:
                    o, l = d, ls[g]
                else:
                    al = jnp.exp2(ms[g - 1] - ms[g])
                    o = o * al + d
                    l = l * al + ls[g]
            outs.append(o * _recip(jnp.sum(l, axis=0, keepdims=True)))
        return outs

    def fin(oa, ob):
        def blk(x, t, n):
            return x[n][t * HB:(t + 1) * HB]
        ca = _strassen_b(blk(oa, 0, 0), blk(oa, 0, 1), blk(oa, 2, 0), blk(oa, 2, 1))
        cb = _strassen_b(blk(ob, 0, 0), blk(ob, 0, 1), blk(ob, 2, 0), blk(ob, 2, 1))
        return [_ipack(ca[i], cb[i]) for i in range(7)] + [_ipack(blk(oa, 1, n), blk(ob, 1, n)) for n in range(NN)]

    def wo_y(os, p):
        sl = _par(p)
        w1 = _unpack(wo1_ref[sl])
        mid = [_dot(w1, _unpack(os[7 + n])) for n in range(NN)]
        c11, c12, c21, c22 = _strassen_c([_dot(_unpack(wos_ref[sl, i]), _unpack(os[i])) for i in range(7)])
        return [jnp.concatenate([c11, c21], axis=0) + mid[0], jnp.concatenate([c12, c22], axis=0) + mid[1]]

    def wo(b, os, p):
        y = wo_y(os, p)
        for n in range(NN):
            acc_ref[:, cols(b, n)] += y[n]

    def epilogue(b, y):
        xs = _iunpack(xt_ref[b])
        outs = []
        for n in range(NN):
            tile = NN * b + n
            off = jnp.where(tile == tile_ref[1], S + 128, jnp.where(tile == tile_ref[0], S, tile * 128))
            hh = jnp.concatenate(_iunpack(xn_ref[:, pl.ds(pl.multiple_of(off, 128), 128)]), axis=0)
            h2 = 0.5 * hh
            g = h2 * jnp.tanh(h2) + h2
            outs.append(xs[n] + (acc_ref[:, cols(b, n)] + y[n]) * g)
        out_buf[cols(b), :] = _unpack(_ipack(outs[0], outs[1]).T)
        cp_out(b).start()

    def router_ffn():
        r = r_ref[...]
        col = lax.broadcasted_iota(I32, (1, S), 1)
        cid = (col // M) * M + 2 * (col % 128) + (col // 128) % 2
        m1 = jnp.max(r, axis=1, keepdims=True)
        i1 = jnp.min(jnp.where(r == m1, cid, S), axis=1, keepdims=True)
        r2 = jnp.where(cid == i1, -jnp.inf, r)
        m2 = jnp.max(r2, axis=1, keepdims=True)
        i2 = jnp.min(jnp.where(jnp.logical_and(r2 == m2, cid != i1), cid, S), axis=1, keepdims=True)
        tok = [jnp.min(jnp.minimum(i1, S - 1)), jnp.min(jnp.minimum(i2, S - 1))]

        def gather(sc):
            base = pl.multiple_of((sc // 16) * 16, 16)
            blk = x_buf[pl.ds(base, 16), :].astype(F32)
            sub = lax.broadcasted_iota(I32, (16, 1), 0)
            xr = jnp.sum(jnp.where(sub == sc % 16, blk, 0.0), axis=0, keepdims=True)
            mu = jnp.sum(xr, axis=1, keepdims=True) * (1.0 / D)
            xc = xr - mu
            var = jnp.sum(xc * xc, axis=1, keepdims=True) * (1.0 / D)
            return _rb(xr - _rb(mu)) * _inv_std(var)
        row = lax.broadcasted_iota(I32, (16, 1), 0)
        xs = jnp.where(row == 0, gather(tok[0]), jnp.where(row == 1, gather(tok[1]), 0.0)).astype(BF16)
        g = _rb(_dot(xs, wg_buf[...]))
        g = _rb(g * _sigmoid(g))
        u = _rb(_dot(xs, wu_buf[...]))
        gu = (g * u).astype(BF16)
        y = _rb(_dot(gu, wd_buf[...]))
        rs = _rb(_sigmoid(jnp.where(row == 0, m1, m2)))
        upd = _rb(y * rs)
        updt = jnp.concatenate([upd, jnp.zeros((112, D), F32)], axis=0).T
        lane = lax.broadcasted_iota(I32, (1, 128), 1)
        tiles = [NN * (t // M) + t % 2 for t in tok]
        for t in range(2):
            src_off = tiles[t] * 128
            if t == 1:
                src_off = jnp.where(tiles[1] == tiles[0], S, src_off)
            lo, hi = _iunpack(xn_ref[:, pl.ds(pl.multiple_of(src_off, 128), 128)])
            add = jnp.where(lane == (tok[t] % M) // 2, updt[:, t:t + 1], 0.0)
            xn_ref[:, S + t * 128:S + (t + 1) * 128] = _ipack(lo + add[:DL], hi + add[DL:])
            tile_ref[t] = tiles[t]

    @pl.when(j == 0)
    def _():
        w0, w1 = cp_w(0), cp_w(1)
        cp_r = pltpu.make_async_copy(wr_hbm, wr_ref, sem_r.at[0])
        cp_x(0).start(); cp_r.start(); w0[0].start()
        acc_ref[...] = jnp.zeros(acc_ref.shape, F32)
        oc_ref[...] = jnp.zeros(oc_ref.shape, U32)
        wos_ref[1] = jnp.zeros(wos_ref.shape[1:], U32)
        wo1_ref[1] = jnp.zeros(wo1_ref.shape[1:], U32)
        cp_r.wait()
        cp_x(1).start(); w0[1].start(); cp_x(2).start(); cp_x(3).start()
        wrc_ref[...] = jnp.broadcast_to(wr_ref[...].astype(F32).reshape(1, D), (128, D)).T
        cp_x(0).wait()
        w0[2].start(); w0[3].start()
        for i in range(4, NQ):
            cp_x(i).start()
        layernorm(0)
        w0[0].wait()
        for c in w1:
            c.start()
        stage_wq(0)
        X0 = qproj(0, 0)
        for t in range(6):
            qc_ref[t] = X0[t]
        w0[1].wait()
        for h in range(2):
            for t in range(3):
                stage_k(0, h, t)

        def ln(i, c):
            cp_x(i).wait()
            layernorm(i)
            return c
        lax.fori_loop(1, 5, ln, 0)
        w0[2].wait()
        stage_wo(0)
        w0[3].wait()
        stage_v(0, 0); stage_v(0, 1)
        lax.fori_loop(5, NQ, ln, 0)

    @pl.when(j + 1 < NPAIR)
    def _():
        for c in cp_w(j + 1):
            c.wait()

    @pl.when(j == 0)
    def _():
        for k in range(3):
            cp_f(k).start()

    @pl.when(j + 2 < NPAIR)
    def _():
        for c in cp_w(j + 2):
            c.start()

    @pl.when(j == 1)
    def _():
        for k in range(3):
            cp_f(k).wait()
        router_ffn()

    def body(last_step):
        X = [qc_ref[t] for t in range(6)]
        o_prev = [oc_ref[t] for t in range(NO)]
        for i in range(NQ):
            last = i == NQ - 1
            if not last_step:
                if i == 3:
                    stage_v(j + 1, 0); stage_v(j + 1, 1)
                if last:
                    stage_wq(j + 1); stage_wo(j + 1)
                    for h in range(2):
                        for t in range(3):
                            stage_k(j + 1, h, t)
            ra = qk_softmax(X, 0, j)
            rb = qk_softmax(X, 1, j)
            if i == 0:
                wo(NQ - 1, o_prev, j + 1)
            elif last_step:
                epilogue(i - 1, wo_y(o_prev, j))
                if last:
                    cp_out(0).wait()
            else:
                wo(i - 1, o_prev, j)
            oa = pv(ra, 0, j)
            if not last:
                X = qproj(i + 1, j)
            elif not last_step:
                Xn = qproj(0, j + 1)
                for t in range(6):
                    qc_ref[t] = Xn[t]
            ob = pv(rb, 1, j)
            o_prev = fin(oa, ob)
        if last_step:
            epilogue(NQ - 1, wo_y(o_prev, j))
            for i in range(1, NQ):
                cp_out(i).wait()
        else:
            for t in range(NO):
                oc_ref[t] = o_prev[t]

    @pl.when(j < NPAIR - 1)
    def _():
        body(False)

    @pl.when(j == NPAIR - 1)
    def _():
        body(True)


@jax.jit
def pallas_recurrent_scan__sliding_block_cached__moe_arch_mod__prompt_kernel(
        A_x, A_k_cache, A_v_cache, A_wq, A_wo, B_x, B_w_r, B_w_gate, B_w_up, B_w_down):
    x = A_x.reshape(S, D)
    kt = jnp.swapaxes(A_k_cache, 2, 3)
    vt = jnp.swapaxes(A_v_cache, 2, 3)
    anyspec = pl.BlockSpec(memory_space=pl.ANY)
    out = pl.pallas_call(
        _kernel,
        grid=(NPAIR,),
        in_specs=[anyspec] * 9,
        out_specs=anyspec,
        out_shape=jax.ShapeDtypeStruct((S, D), BF16),
        scratch_shapes=[
            pltpu.VMEM((S, D), BF16),
            pltpu.VMEM((NQ, D, 128), U32),
            pltpu.VMEM((DL, S + 256), U32),
            pltpu.VMEM((NQ, 5, 128, 128), U32),
            pltpu.VMEM((D, S), F32),
            pltpu.VMEM((2, D, PW), BF16),
            pltpu.VMEM((2, PW, D), BF16),
            pltpu.VMEM((2, 2, DH, W), BF16),
            pltpu.VMEM((2, 2, DH, W), BF16),
            pltpu.VMEM((2, 7, DH // 2, 256), U32),
            pltpu.VMEM((2, PW // 2, 128), U32),
            pltpu.VMEM((2, 2, 3, KH // 2, 128), U32),
            pltpu.VMEM((2, 2, G, DH // 2, 128), U32),
            pltpu.VMEM((2, 7, DL // 2, 128), U32),
            pltpu.VMEM((2, DL, 128), U32),
            pltpu.VMEM((6, HB, M), U32),
            pltpu.VMEM((NO, HB, 128), U32),
            pltpu.VMEM((1, S), F32),
            pltpu.SMEM((2,), I32),
            pltpu.VMEM((D, FF), BF16),
            pltpu.VMEM((D, FF), BF16),
            pltpu.VMEM((FF, D), BF16),
            pltpu.VMEM((S, D), BF16),
            pltpu.VMEM((KH, 128), F32),
            pltpu.VMEM((D, 128), F32),
            pltpu.VMEM((D,), BF16),
            pltpu.SemaphoreType.DMA((NQ,)),
            pltpu.SemaphoreType.DMA((8,)),
            pltpu.SemaphoreType.DMA((3,)),
            pltpu.SemaphoreType.DMA((NQ,)),
            pltpu.SemaphoreType.DMA((1,)),
        ],
        compiler_params=pltpu.CompilerParams(
            dimension_semantics=("arbitrary",),
            vmem_limit_bytes=100 * 1024 * 1024,
            disable_bounds_checks=True),
        name="fused_attn_mod",
    )(x, kt, vt, A_wq, A_wo, B_w_r, B_w_gate, B_w_up, B_w_down)
    return out.reshape(1, S, D)
```
